```python
import os as _os
_os.environ.setdefault("JAX_PLATFORMS", "cpu")
import jax
import jax.numpy as jnp

def _softmax(x, axis=-1):
    return jax.nn.softmax(x, axis=axis)
def _gelu(x):
    return jax.nn.gelu(x, approximate=True)
def _silu(x):
    return jax.nn.silu(x)
def _sigmoid(x):
    return jax.nn.sigmoid(x)
def _layernorm(x, axis=-1, eps=1e-5):
    m = jnp.mean(x, axis=axis, keepdims=True)
    v = jnp.var(x, axis=axis, keepdims=True)
    return (x - m) / jnp.sqrt(v + eps)
def _scatter_add(tgt, idx, src, axis=0):
    return tgt.at[idx].add(src)
def _segment_sum(src, seg, n):
    return jax.ops.segment_sum(src, seg, n)
class _Rng:
    def __init__(self, key):
        self._k = key
    def _next(self):
        self._k, sub = jax.random.split(self._k)
        return sub
    def normal(self, shape):
        return jax.random.normal(self._next(), shape, dtype=jnp.bfloat16)
    def randint(self, lo, hi, shape):
        return jax.random.randint(self._next(), shape, lo, hi, dtype=jnp.int32)
    def uniform(self, shape, lo=0.0, hi=1.0):
        return jax.random.uniform(self._next(), shape, jnp.bfloat16, lo, hi)
    def permutation(self, n):
        return jax.random.permutation(self._next(), n)


kernel_name = 'gated_mix__softmax_full_mha__dense_activation_relu__prompt'

def setup_inputs():
    _rng = _Rng(jax.random.key(int.from_bytes(__import__("os").urandom(4), "little")))
    _w = (lambda a: (lambda t: t.astype(jnp.bfloat16) if jnp.issubdtype(t.dtype, jnp.floating) else t)(jnp.asarray(a)))
    def _A_setup():
        B, S, D = 1, 2048, 640
        return {
            "x": _w((lambda *s: _rng.normal(s) * 0.05)(B, S, D)),
            "wqkv": _w((lambda *s: _rng.normal(s) * 0.8)(D, 3 * D)),
            "wo": _w((lambda *s: _rng.normal(s) * 0.05)(D, D)),
        }
    _A_in = _A_setup()

    def _B_setup():
        B, S, D, Dff = 1, 2048, 640, 1536
        return {
            "x": _w((lambda *s: _rng.normal(s) * 0.05)(B, S, D)),
            "w1": _w((lambda *s: _rng.normal(s) * 0.05)(D, Dff)),
            "w2": _w((lambda *s: _rng.normal(s) * 0.05)(Dff, D)),
        }
    _B_in = _B_setup()

    return {
        "A_x": _A_in["x"],
        "A_wqkv": _A_in["wqkv"],
        "A_wo": _A_in["wo"],
        "B_x": _B_in["x"],
        "B_w1": _B_in["w1"],
        "B_w2": _B_in["w2"],
        "gate_w": _w((lambda *s: _rng.normal(s) * 0.05)(640) * 16.0),
    }

def reference(A_x, A_wqkv, A_wo, B_x, B_w1, B_w2, gate_w):
    def _A_ref(x, wqkv, wo):
        B, S, D = x.shape
        H = 32; Dh = D // H
        qkv = (lambda x, *d: x.transpose(*d))((x @ wqkv).reshape(B, S, 3, H, Dh), 2, 0, 3, 1, 4)
        q, k, v = qkv[0], qkv[1], qkv[2]
        scale = Dh ** -0.5
        scores = jnp.einsum("bhqd,bhkd->bhqk", q, k) * scale
        p = _softmax(scores, axis=-1)
        o = jnp.einsum("bhqk,bhkd->bhqd", p, v)
        return (lambda x, *d: x.transpose(*d))(o, 0, 2, 1, 3).reshape(B, S, D) @ wo

    def _B_ref(x, w1, w2):
        h = jnp.einsum("bsd,df->bsf", x, w1)
        zero = jnp.zeros_like(h)
        h = jnp.maximum(h, zero)
        return jnp.einsum("bsf,fd->bsd", h, w2)

    x = A_x
    g = _sigmoid((x * gate_w).sum(-1, keepdims=True))
    a = _A_ref(x, A_wqkv, A_wo)
    b = _B_ref(x, B_w1, B_w2)
    return g * a + (1 - g) * b
```

```python
import math
import jax
import jax.numpy as jnp
import jax.experimental.pallas as pl
import jax.experimental.pallas.tpu as pltpu

S, D, H, DH, DFF = 2048, 640, 32, 20, 1536
NT = D // 128
F32, BF16, U32 = jnp.float32, jnp.bfloat16, jnp.uint32
STRADDLE = [h for h in range(H) if (h * DH) // 128 != (h * DH + DH - 1) // 128]
NN = (((1,), (0,)), ((), ()))
NTR = (((1,), (1,)), ((), ()))

def dot(a, b, dims=NN):
    return jax.lax.dot_general(a, b, dims, preferred_element_type=F32)

def pack(v):
    return pltpu.bitcast(v.astype(BF16), U32)

def make(BQ=512, KC=128, G=1, RB=512, order='dqv', loop1=True, loop3=True, flags=None, cfin=4, cq_=8, nsteps=None):
    NQ = S // BQ
    T = NQ * H
    NC = S // KC
    NR = S // RB
    cq = (DH ** -0.5) * math.log2(math.e)

    def kernel(x_hbm, wqkv_hbm, wo_hbm, w1_hbm, w2_hbm, gw_ref, out_hbm,
               x_ref, wq_ref, wk_ref, wv_ref, wo_ref, w1_ref, w2_ref, o_buf, wqT_ref, wvT_ref,
               k_scr, qt_scr, vt_scr, ot_scr, s_scr, q_cur, acc_scr, xsem, wsem, osem):
        def xcopy(r):
            return pltpu.make_async_copy(x_hbm.at[pl.ds(r * RB, RB), :], x_ref.at[pl.ds(r * RB, RB), :], xsem.at[r])
        wcopies = [
            pltpu.make_async_copy(wqkv_hbm.at[:, D:2 * D], wk_ref, wsem.at[0]),
            pltpu.make_async_copy(wqkv_hbm.at[:, 0:D], wq_ref, wsem.at[1]),
            pltpu.make_async_copy(wqkv_hbm.at[:, 2 * D:3 * D], wv_ref, wsem.at[2]),
            pltpu.make_async_copy(w1_hbm, w1_ref, wsem.at[3]),
            pltpu.make_async_copy(w2_hbm, w2_ref, wsem.at[4]),
            pltpu.make_async_copy(wo_hbm, wo_ref, wsem.at[5]),
        ]
        xcopy(0).start()
        wcopies[0].start()

        lane = jax.lax.broadcasted_iota(jnp.int32, (RB, 128), 1)
        row128 = jax.lax.broadcasted_iota(jnp.int32, (128, RB), 0)
        row8 = jax.lax.broadcasted_iota(jnp.int32, (8, RB), 0)

        def rows(r, n):
            return pl.ds(r * n if isinstance(r, int) else pl.multiple_of(r * n, n), n)

        def kproj(r):
            k = dot(x_ref[rows(r, RB), :], wk_ref[...])
            for t in range(NT):
                k_scr[t, rows(r, RB // 2), :] = pack(k[:, t * 128:(t + 1) * 128])
            for i, h in enumerate(STRADDLE):
                t, lo = divmod(h * DH, 128)
                k_scr[NT + i, rows(r, RB // 2), :] = pack(jnp.where(
                    lane >= lo, k[:, t * 128:(t + 1) * 128], k[:, (t + 1) * 128:(t + 2) * 128]))

        def qvproj(r):
            xs = x_ref[rows(r, RB), :]
            qT = dot(pltpu.bitcast(wqT_ref[...], BF16), xs, NTR) * cq
            for t in range(NT):
                qt_scr[t, :, rows(r, RB)] = pack(qT[t * 128:(t + 1) * 128, :])
            for i, h in enumerate(STRADDLE):
                t, lo = divmod(h * DH, 128)
                qt_scr[NT + i, :, rows(r, RB)] = pack(jnp.where(
                    row128 >= lo, qT[t * 128:(t + 1) * 128, :], qT[(t + 1) * 128:(t + 2) * 128, :]))
            vT = dot(pltpu.bitcast(wvT_ref[...], BF16), xs, NTR).astype(BF16).astype(F32)
            for p in range(H // 2):
                b = 40 * p
                mid = vT[b + 16:b + 24, :]
                vt_scr[2 * p, 0:16, rows(r, RB)] = vT[b:b + 16, :]
                vt_scr[2 * p, 16:24, rows(r, RB)] = jnp.where(row8 < 4, mid, 1.0)
                vt_scr[2 * p + 1, 0:8, rows(r, RB)] = jnp.where(row8 < 4, 1.0, mid)
                vt_scr[2 * p + 1, 8:24, rows(r, RB)] = vT[b + 24:b + 40, :]

        def run(f, n, loop):
            if loop:
                jax.lax.fori_loop(0, n, lambda i, c: (f(i), c)[1], 0)
            else:
                for i in range(n):
                    f(i)

        wcopies[0].wait()
        xcopy(0).wait()
        for r in range(1, NR // 2):
            xcopy(r).start()
        for r in range(NR // 2):
            if r > 0:
                xcopy(r).wait()
            if r == NR // 4:
                for r2 in range(NR // 2, NR):
                    xcopy(r2).start()
                wcopies[1].start()
                wcopies[2].start()
            kproj(r)
        for r in range(NR // 2, NR):
            xcopy(r).wait()
        wcopies[1].wait()
        wcopies[2].wait()
        for c in wcopies[3:]:
            c.start()
        for r in range(NR // 2, NR):
            kproj(r)
            if r == NR // 2:
                wqT_ref[...] = pack(wq_ref[...].astype(F32).T)
            if r == NR // 2 + NR // 4 - (1 if NR > 4 else 0):
                wvT_ref[...] = pack(wv_ref[...].astype(F32).T)
        run(qvproj, NR, loop1)

        rowp = jax.lax.broadcasted_iota(jnp.int32, (64, BQ), 0)
        r24 = jax.lax.broadcasted_iota(jnp.int32, (24, BQ), 0)

        def tile_of(t):
            h = t % H
            tile = (h * DH) // 128
            for i, hs in enumerate(STRADDLE):
                tile = jnp.where(h == hs, NT + i, tile)
            return tile

        def prep_q(t, g):
            t = jnp.minimum(t, T - 1)
            lo2 = (((t % H) * DH) % 128) // 2
            q = qt_scr[tile_of(t), :, rows(t // H, BQ)]
            return jnp.where(((rowp - lo2) & 63) < DH // 2, q, jnp.uint32(0))

        def qk_chunk(g, tile, q, c):
            s = dot(pltpu.bitcast(k_scr[tile, c * KC // 2:(c + 1) * KC // 2, :], BF16), q)
            s_scr[g, c * KC:(c + 1) * KC, :] = s
            return jnp.max(s.reshape(KC // 8, 8, BQ), axis=0)

        def finish(t, g):
            t = jnp.maximum(t, 0)
            h = t % H
            odd = h % 2
            acc = acc_scr[g]
            l = jnp.where(odd == 1, acc[0:1, :], acc[23:24, :])
            o = acc * (1.0 / l)
            dst = (pl.ds(pl.multiple_of((h // 2) * 40 + odd * 16, 8), 24), rows(t // H, BQ))
            keep = r24 < 4 * odd
            ot_scr[dst] = jnp.where(keep, ot_scr[dst], o)

        ms = []
        ot_scr[0:24, 0:BQ] = jnp.zeros((24, BQ), F32)
        for g in range(G):
            t = jnp.int32(g)
            q = pltpu.bitcast(prep_q(t, g), BF16)
            m = None
            for c in range(NC):
                mc = qk_chunk(g, tile_of(t), q, c)
                m = mc if m is None else jnp.maximum(m, mc)
            ms.append(jnp.max(m, axis=0, keepdims=True))
            q_cur[g] = prep_q(t + G, g)
            acc_scr[g] = jnp.ones((24, BQ), F32)

        def body(j, carry, last=False, extra=None):
            ms, tiles = carry
            new_ms, new_tiles = [], []
            for g in range(G):
                t = j * G + g
                h = t % H
                m = ms[g]
                q = pltpu.bitcast(q_cur[g], BF16)
                acc, mn = None, None
                for c in range(NC):
                    for ch in order:
                        if ch == 'd':
                            p = jnp.exp2(s_scr[g, c * KC:(c + 1) * KC, :] - m).astype(BF16)
                        elif ch == 'v':
                            a = dot(vt_scr[h, :, c * KC:(c + 1) * KC], p)
                            acc = a if acc is None else acc + a
                        elif ch == 'q' and not last:
                            mc = qk_chunk(g, tiles[g], q, c)
                            mn = mc if mn is None else jnp.maximum(mn, mc)
                    if c == cfin:
                        finish(t - G, g)
                    if c == cq_ and not last:
                        qn = prep_q(t + 2 * G, g)
                acc_scr[g] = acc
                if last:
                    continue
                q_cur[g] = qn
                new_ms.append(jnp.max(mn, axis=0, keepdims=True))
                new_tiles.append(tile_of(jnp.minimum(t + 2 * G, T - 1)))
            return tuple(new_ms), tuple(new_tiles)
        carry = jax.lax.fori_loop(0, (nsteps or T) // G - 1, body, (tuple(ms), tuple(tile_of(jnp.int32(G + g)) for g in range(G))))
        body(jnp.int32(T // G - 1), carry, last=True)
        for g in range(G):
            finish(jnp.int32(T - G + g), g)

        for c in wcopies[3:]:
            c.wait()
        gw = gw_ref[...].astype(F32).reshape(1, D)
        def ocopy(r):
            return pltpu.make_async_copy(o_buf.at[rows(r, RB), :], out_hbm.at[rows(r, RB), :], osem.at[r])
        def final(r):
            xs = x_ref[rows(r, RB), :]
            hh = jnp.maximum(dot(xs, w1_ref[...]), 0.0).astype(BF16)
            g = jax.nn.sigmoid(jnp.sum(xs.astype(F32) * gw, axis=-1, keepdims=True))
            o = ot_scr[:, rows(r, RB)].T.astype(BF16)
            b = dot(hh, w2_ref[...])
            a = dot(o, wo_ref[...])
            o_buf[rows(r, RB), :] = (g * a + (1.0 - g) * b).astype(o_buf.dtype)
            ocopy(r).start()
        run(final, NR, loop3)
        for r in range(NR):
            ocopy(r).wait()

    def fn(A_x, A_wqkv, A_wo, B_x, B_w1, B_w2, gate_w):
        anyspec = pl.BlockSpec(memory_space=pl.ANY)
        out = pl.pallas_call(
            kernel,
            out_shape=jax.ShapeDtypeStruct((S, D), A_x.dtype),
            in_specs=[anyspec] * 5 + [pl.BlockSpec(memory_space=pltpu.VMEM)],
            out_specs=anyspec,
            scratch_shapes=[
                pltpu.VMEM((S, D), BF16), pltpu.VMEM((D, D), BF16), pltpu.VMEM((D, D), BF16), pltpu.VMEM((D, D), BF16),
                pltpu.VMEM((D, D), BF16), pltpu.VMEM((D, DFF), BF16), pltpu.VMEM((DFF, D), BF16),
                pltpu.VMEM((S, D), BF16),
                pltpu.VMEM((D // 2, D), U32), pltpu.VMEM((D // 2, D), U32),
                pltpu.VMEM((NT + 4, S // 2, 128), U32),
                pltpu.VMEM((NT + 4, 64, S), U32),
                pltpu.VMEM((H, 24, S), F32),
                pltpu.VMEM((D, S), F32),
                pltpu.VMEM((G, S, BQ), F32),
                pltpu.VMEM((G, 64, BQ), U32),
                pltpu.VMEM((G, 24, BQ), F32),
                pltpu.SemaphoreType.DMA((NR,)), pltpu.SemaphoreType.DMA((6,)), pltpu.SemaphoreType.DMA((NR,)),
            ],
            compiler_params=pltpu.CompilerParams(vmem_limit_bytes=100 * 1024 * 1024, flags=flags),
        )(A_x.reshape(S, D), A_wqkv, A_wo, B_w1, B_w2, gate_w)
        return out.reshape(1, S, D)
    return jax.jit(fn)


_fn = make(**{'G':4,'RB':256,'loop1':False})

@jax.jit
def pallas_gated_mix__softmax_full_mha__dense_activation_relu__prompt_kernel(A_x, A_wqkv, A_wo, B_x, B_w1, B_w2, gate_w):
    return _fn(A_x, A_wqkv, A_wo, B_x, B_w1, B_w2, gate_w)
```

```python
import math

import jax
import jax.numpy as jnp
import jax.experimental.pallas as pl
import jax.experimental.pallas.tpu as pltpu

S, D, H, DH, DFF = 2048, 640, 32, 20, 1536
F32, BF16, U32 = jnp.float32, jnp.bfloat16, jnp.uint32

BQ = 512
KC = 128
G = 4
RB = 256
XCH = (384, 896, 768)
NQ, NC, NR = S // BQ, S // KC, S // RB
T = NQ * H
NT = D // 128
STRADDLE = [h for h in range(H) if (h * DH) // 128 != (h * DH + DH - 1) // 128]
NX = NT + len(STRADDLE)
QSCALE = DH ** -0.5 * math.log2(math.e)


def _dot(a, b, rhs_dim=0):
    return jax.lax.dot_general(a, b, (((1,), (rhs_dim,)), ((), ())), preferred_element_type=F32)


def _pack(v):
    return pltpu.bitcast(v.astype(BF16), U32)


def _unpack(v):
    return pltpu.bitcast(v, BF16)


def _rows(r, n):
    return pl.ds(r * n if isinstance(r, int) else pl.multiple_of(r * n, n), n)


def _kernel(x_hbm, wqkv_hbm, wo_hbm, w1_hbm, w2_hbm, gw_ref, out_hbm,
            x_ref, wq_ref, wk_ref, wv_ref, wo_ref, w1_ref, w2_ref, o_buf, wqT_ref, wvT_ref,
            k_scr, qt_scr, vt_scr, ot_scr, s_scr, q_cur, q_nxt, acc_scr, xsem, wsem, osem):
    def xcopy(r):
        sl = pl.ds(sum(XCH[:r]), XCH[r])
        return pltpu.make_async_copy(x_hbm.at[sl, :], x_ref.at[sl, :], xsem.at[r])

    wk_copy = pltpu.make_async_copy(wqkv_hbm.at[:, D:2 * D], wk_ref, wsem.at[0])
    wq_copy = pltpu.make_async_copy(wqkv_hbm.at[:, 0:D], wq_ref, wsem.at[1])
    wv_copy = pltpu.make_async_copy(wqkv_hbm.at[:, 2 * D:3 * D], wv_ref, wsem.at[2])
    late_copies = [
        pltpu.make_async_copy(w1_hbm, w1_ref, wsem.at[3]),
        pltpu.make_async_copy(w2_hbm, w2_ref, wsem.at[4]),
        pltpu.make_async_copy(wo_hbm, wo_ref, wsem.at[5]),
    ]

    def kproj(a, n):
        k = _dot(x_ref[a:a + n, :], wk_ref[...])
        lane = jax.lax.broadcasted_iota(jnp.int32, (n, 128), 1)
        for t in range(NT):
            k_scr[t, a // 2:(a + n) // 2, :] = _pack(k[:, t * 128:(t + 1) * 128])
        for i, h in enumerate(STRADDLE):
            t, lo = divmod(h * DH, 128)
            k_scr[NT + i, a // 2:(a + n) // 2, :] = _pack(jnp.where(
                lane >= lo, k[:, t * 128:(t + 1) * 128], k[:, (t + 1) * 128:(t + 2) * 128]))

    def qvproj(r):
        row128 = jax.lax.broadcasted_iota(jnp.int32, (128, RB), 0)
        row8 = jax.lax.broadcasted_iota(jnp.int32, (8, RB), 0)
        xs = x_ref[_rows(r, RB), :]
        qT = _dot(_unpack(wqT_ref[...]), xs, 1) * QSCALE
        for t in range(NT):
            qt_scr[t, :, _rows(r, RB)] = _pack(qT[t * 128:(t + 1) * 128, :])
        for i, h in enumerate(STRADDLE):
            t, lo = divmod(h * DH, 128)
            qt_scr[NT + i, :, _rows(r, RB)] = _pack(jnp.where(
                row128 >= lo, qT[t * 128:(t + 1) * 128, :], qT[(t + 1) * 128:(t + 2) * 128, :]))
        for g in range(G):
            k_scr[NX + g, _rows(r, RB // 2), :] = _pack(xs[:, g * 128:(g + 1) * 128])
        vT = _dot(_unpack(wvT_ref[...]), xs, 1).astype(BF16).astype(F32)
        for p in range(H // 2):
            b = 2 * DH * p
            mid = vT[b + 16:b + 24, :]
            vt_scr[2 * p, 0:16, _rows(r, RB)] = vT[b:b + 16, :]
            vt_scr[2 * p, 16:24, _rows(r, RB)] = jnp.where(row8 < 4, mid, 1.0)
            vt_scr[2 * p + 1, 0:8, _rows(r, RB)] = jnp.where(row8 < 4, 1.0, mid)
            vt_scr[2 * p + 1, 8:24, _rows(r, RB)] = vT[b + 24:b + 40, :]

    xcopy(0).start()
    wk_copy.start()
    wk_copy.wait()
    xcopy(0).wait()
    for r in range(1, len(XCH)):
        xcopy(r).start()
    wq_copy.start()
    wv_copy.start()
    for r in range(len(XCH)):
        if r > 0:
            xcopy(r).wait()
        if r == len(XCH) - 1:
            wq_copy.wait()
            wv_copy.wait()
            for c in late_copies:
                c.start()
            wqT_ref[...] = _pack(wq_ref[...].astype(F32).T)
        for b in range(0, XCH[r], RB):
            kproj(sum(XCH[:r]) + b, min(RB, XCH[r] - b))
    wvT_ref[...] = _pack(wv_ref[...].astype(F32).T)
    for r in range(NR):
        qvproj(r)

    rowpair = jax.lax.broadcasted_iota(jnp.int32, (64, BQ), 0)
    row8q = jax.lax.broadcasted_iota(jnp.int32, (8, BQ), 0)

    def tile_of(t):
        h = t % H
        tile = (h * DH) // 128
        for i, hs in enumerate(STRADDLE):
            tile = jnp.where(h == hs, NT + i, tile)
        return jnp.where(t >= T, NX + t % G, tile)

    def masked_q(t):
        lo2 = (((t % H) * DH) % 128) // 2
        q = qt_scr[tile_of(t), :, _rows((t // H) % NQ, BQ)]
        return jnp.where(((rowpair - lo2) & 63) < jnp.where(t >= T, 64, DH // 2), q, jnp.uint32(0))

    def scores(g, tile, q, c):
        s = _dot(_unpack(k_scr[tile, c * KC // 2:(c + 1) * KC // 2, :]), q)
        s_scr[g, c * KC:(c + 1) * KC, :] = s
        return jnp.max(s.reshape(KC // 8, 8, BQ), axis=0)

    def finish(t, odd, acc):
        base = ((t % H) // 2) * 2 * DH
        cols = _rows(t // H, BQ)
        if odd:
            o = acc * (1.0 / acc[0:1, :])
            shared = pl.ds(pl.multiple_of(base + 16, 8), 8)
            ot_scr[shared, cols] = jnp.where(row8q < 4, ot_scr[shared, cols], o[0:8])
            ot_scr[pl.ds(pl.multiple_of(base + 24, 8), 16), cols] = o[8:24]
        else:
            ot_scr[pl.ds(pl.multiple_of(base, 8), 24), cols] = acc * (1.0 / acc[23:24, :])

    ms = []
    for g in range(G):
        t = jnp.int32(g)
        q = _unpack(masked_q(t))
        m = None
        for c in range(NC):
            mc = scores(g, tile_of(t), q, c)
            m = mc if m is None else jnp.maximum(m, mc)
        ms.append(jnp.max(m, axis=0, keepdims=True))
        q_cur[g] = masked_q(t + G)
    q_nxt[G - 1] = q_cur[G - 1]
    acc_scr[...] = jnp.ones((24, BQ), F32)
    ot_scr[16:24, 0:BQ] = jnp.zeros((8, BQ), F32)

    for c in late_copies:
        c.wait()
    for g in range(G):
        qt_scr[NX + g, :, 0:BQ] = _pack(w1_ref[g * 128:(g + 1) * 128, 0:BQ])

    def body(j, carry):
        ms, tiles = carry
        new_ms, new_tiles = [], []
        acc = None
        for g in range(G):
            t = j * G + g
            h = t % H
            q = _unpack(q_cur[g])
            prev, acc, mn = acc, None, None
            for c in range(NC):
                p = jnp.exp2(s_scr[g, c * KC:(c + 1) * KC, :] - ms[g]).astype(BF16)
                mc = scores(g, tiles[g], q, c)
                mn = mc if mn is None else jnp.maximum(mn, mc)
                a = _dot(vt_scr[h, :, c * KC:(c + 1) * KC], p)
                acc = a if acc is None else acc + a
                if c == 4:
                    if g == 0:
                        finish(jnp.maximum(t - 1, 1), True, acc_scr[...])
                    else:
                        finish(t - 1, g % 2 == 0, prev)
                if c == 8:
                    q_nxt[g] = masked_q(t + 2 * G)
                if c == 12:
                    q_cur[(g - 1) % G] = q_nxt[(g - 1) % G]
            new_ms.append(jnp.max(mn, axis=0, keepdims=True))
            new_tiles.append(tile_of(t + 2 * G))
        acc_scr[...] = acc
        return tuple(new_ms), tuple(new_tiles)

    jax.lax.fori_loop(0, T // G, body,
                      (tuple(ms), tuple(tile_of(jnp.int32(G + g)) for g in range(G))))
    finish(jnp.int32(T - 1), True, acc_scr[...])

    gw = gw_ref[...].astype(F32).reshape(1, D)

    def ocopy(r):
        return pltpu.make_async_copy(o_buf.at[_rows(r, RB), :], out_hbm.at[_rows(r, RB), :], osem.at[r])

    def final(r, carry):
        xs = x_ref[_rows(r, RB), :]
        h1 = _dot(xs, w1_ref[:, BQ:])
        h0 = _dot(xs[:, G * 128:], w1_ref[G * 128:, 0:BQ])
        for g in range(G):
            h0 = h0 + s_scr[g, _rows(r, RB), :]
        hid = jnp.maximum(jnp.concatenate([h0, h1], axis=1), 0.0).astype(BF16)
        gate = jax.nn.sigmoid(jnp.sum(xs.astype(F32) * gw, axis=-1, keepdims=True))
        o = ot_scr[:, _rows(r, RB)].T.astype(BF16)
        b = _dot(hid, w2_ref[...])
        a = _dot(o, wo_ref[...])
        o_buf[_rows(r, RB), :] = (gate * a + (1.0 - gate) * b).astype(o_buf.dtype)
        ocopy(r).start()
        return carry

    jax.lax.fori_loop(0, NR, final, 0)
    for r in range(NR):
        ocopy(r).wait()


@jax.jit
def pallas_gated_mix__softmax_full_mha__dense_activation_relu__prompt_kernel(
    A_x: jax.Array,
    A_wqkv: jax.Array,
    A_wo: jax.Array,
    B_x: jax.Array,
    B_w1: jax.Array,
    B_w2: jax.Array,
    gate_w: jax.Array,
):
    del B_x
    hbm = pl.BlockSpec(memory_space=pl.ANY)
    out = pl.pallas_call(
        _kernel,
        out_shape=jax.ShapeDtypeStruct((S, D), A_x.dtype),
        in_specs=[hbm] * 5 + [pl.BlockSpec(memory_space=pltpu.VMEM)],
        out_specs=hbm,
        scratch_shapes=[
            pltpu.VMEM((S, D), BF16),
            pltpu.VMEM((D, D), BF16),
            pltpu.VMEM((D, D), BF16),
            pltpu.VMEM((D, D), BF16),
            pltpu.VMEM((D, D), BF16),
            pltpu.VMEM((D, DFF), BF16),
            pltpu.VMEM((DFF, D), BF16),
            pltpu.VMEM((S, D), BF16),
            pltpu.VMEM((D // 2, D), U32),
            pltpu.VMEM((D // 2, D), U32),
            pltpu.VMEM((NX + G, S // 2, 128), U32),
            pltpu.VMEM((NX + G, 64, S), U32),
            pltpu.VMEM((H, 24, S), F32),
            pltpu.VMEM((D, S), F32),
            pltpu.VMEM((G, S, BQ), F32),
            pltpu.VMEM((G, 64, BQ), U32),
            pltpu.VMEM((G, 64, BQ), U32),
            pltpu.VMEM((24, BQ), F32),
            pltpu.SemaphoreType.DMA((len(XCH),)),
            pltpu.SemaphoreType.DMA((6,)),
            pltpu.SemaphoreType.DMA((NR,)),
        ],
        compiler_params=pltpu.CompilerParams(
            vmem_limit_bytes=100 * 1024 * 1024,
            flags={"XLA_TPU_EVENLY_DISTRIBUTE_CRITICAL_NODES": True},
        ),
    )(A_x.reshape(S, D), A_wqkv, A_wo, B_w1, B_w2, gate_w)
    return out.reshape(1, S, D)
```

```python
import math

import jax
import jax.numpy as jnp
import jax.experimental.pallas as pl
import jax.experimental.pallas.tpu as pltpu

S, D, H, DH, DFF = 2048, 640, 32, 20, 1536
F32, BF16, U32 = jnp.float32, jnp.bfloat16, jnp.uint32

BQ = 512
KC = 128
G = 4
RB = 256
XCH = (384, 896, 768)
NQ, NC, NR = S // BQ, S // KC, S // RB
T = NQ * H
NT = D // 128
STRADDLE = [h for h in range(H) if (h * DH) // 128 != (h * DH + DH - 1) // 128]
NX = NT + len(STRADDLE)
QSCALE = DH ** -0.5 * math.log2(math.e)


def _dot(a, b, rhs_dim=0):
    return jax.lax.dot_general(a, b, (((1,), (rhs_dim,)), ((), ())), preferred_element_type=F32)


def _pack(v):
    return pltpu.bitcast(v.astype(BF16), U32)


def _unpack(v):
    return pltpu.bitcast(v, BF16)


def _rows(r, n):
    return pl.ds(r * n if isinstance(r, int) else pl.multiple_of(r * n, n), n)


def _kernel(x_hbm, wqkv_hbm, wo_hbm, w1_hbm, w2_hbm, gw_hbm, out_hbm,
            gw_ref, x_ref, wq_ref, wk_ref, wv_ref, wo_ref, w1_ref, w2_ref, o_buf, wqT_ref, wvT_ref,
            k_scr, qt_scr, vt_scr, ot_scr, s_scr, q_cur, q_nxt, acc_scr, xsem, wsem, osem):
    def xcopy(r):
        sl = pl.ds(sum(XCH[:r]), XCH[r])
        return pltpu.make_async_copy(x_hbm.at[sl, :], x_ref.at[sl, :], xsem.at[r])

    wk_copy = pltpu.make_async_copy(wqkv_hbm.at[:, D:2 * D], wk_ref, wsem.at[0])
    wq_copy = pltpu.make_async_copy(wqkv_hbm.at[:, 0:D], wq_ref, wsem.at[1])
    wv_copy = pltpu.make_async_copy(wqkv_hbm.at[:, 2 * D:3 * D], wv_ref, wsem.at[2])
    late_copies = [
        pltpu.make_async_copy(w1_hbm, w1_ref, wsem.at[3]),
        pltpu.make_async_copy(w2_hbm, w2_ref, wsem.at[4]),
        pltpu.make_async_copy(wo_hbm, wo_ref, wsem.at[5]),
        pltpu.make_async_copy(gw_hbm, gw_ref, wsem.at[6]),
    ]

    def kproj(a, n):
        k = _dot(x_ref[a:a + n, :], wk_ref[...])
        lane = jax.lax.broadcasted_iota(jnp.int32, (n, 128), 1)
        for t in range(NT):
            k_scr[t, a // 2:(a + n) // 2, :] = _pack(k[:, t * 128:(t + 1) * 128])
        for i, h in enumerate(STRADDLE):
            t, lo = divmod(h * DH, 128)
            k_scr[NT + i, a // 2:(a + n) // 2, :] = _pack(jnp.where(
                lane >= lo, k[:, t * 128:(t + 1) * 128], k[:, (t + 1) * 128:(t + 2) * 128]))

    def qvproj(r):
        row128 = jax.lax.broadcasted_iota(jnp.int32, (128, RB), 0)
        row8 = jax.lax.broadcasted_iota(jnp.int32, (8, RB), 0)
        xs = x_ref[_rows(r, RB), :]
        qT = _dot(_unpack(wqT_ref[...]), xs, 1) * QSCALE
        for t in range(NT):
            qt_scr[t, :, _rows(r, RB)] = _pack(qT[t * 128:(t + 1) * 128, :])
        for i, h in enumerate(STRADDLE):
            t, lo = divmod(h * DH, 128)
            qt_scr[NT + i, :, _rows(r, RB)] = _pack(jnp.where(
                row128 >= lo, qT[t * 128:(t + 1) * 128, :], qT[(t + 1) * 128:(t + 2) * 128, :]))
        for g in range(G):
            k_scr[NX + g, _rows(r, RB // 2), :] = _pack(xs[:, g * 128:(g + 1) * 128])
        vT = _dot(_unpack(wvT_ref[...]), xs, 1).astype(BF16).astype(F32)
        for p in range(H // 2):
            b = 2 * DH * p
            mid = vT[b + 16:b + 24, :]
            vt_scr[2 * p, 0:16, _rows(r, RB)] = vT[b:b + 16, :]
            vt_scr[2 * p, 16:24, _rows(r, RB)] = jnp.where(row8 < 4, mid, 1.0)
            vt_scr[2 * p + 1, 0:8, _rows(r, RB)] = jnp.where(row8 < 4, 1.0, mid)
            vt_scr[2 * p + 1, 8:24, _rows(r, RB)] = vT[b + 24:b + 40, :]

    xcopy(0).start()
    wk_copy.start()
    wk_copy.wait()
    xcopy(0).wait()
    for r in range(1, len(XCH)):
        xcopy(r).start()
    wq_copy.start()
    wv_copy.start()
    for r in range(len(XCH)):
        if r > 0:
            xcopy(r).wait()
        if r == len(XCH) - 1:
            wq_copy.wait()
            wv_copy.wait()
            for c in late_copies:
                c.start()
            wqT_ref[...] = _pack(wq_ref[...].astype(F32).T)
        for b in range(0, XCH[r], RB):
            kproj(sum(XCH[:r]) + b, min(RB, XCH[r] - b))
    wvT_ref[...] = _pack(wv_ref[...].astype(F32).T)
    for r in range(NR):
        qvproj(r)

    rowpair = jax.lax.broadcasted_iota(jnp.int32, (64, BQ), 0)
    row8q = jax.lax.broadcasted_iota(jnp.int32, (8, BQ), 0)

    def tile_of(t):
        h = t % H
        tile = (h * DH) // 128
        for i, hs in enumerate(STRADDLE):
            tile = jnp.where(h == hs, NT + i, tile)
        return jnp.where(t >= T, NX + t % G, tile)

    def masked_q(t):
        lo2 = (((t % H) * DH) % 128) // 2
        q = qt_scr[tile_of(t), :, _rows((t // H) % NQ, BQ)]
        return jnp.where(((rowpair - lo2) & 63) < jnp.where(t >= T, 64, DH // 2), q, jnp.uint32(0))

    def scores(g, tile, q, c):
        s = _dot(_unpack(k_scr[tile, c * KC // 2:(c + 1) * KC // 2, :]), q)
        s_scr[g, c * KC:(c + 1) * KC, :] = s
        return jnp.max(s.reshape(KC // 8, 8, BQ), axis=0)

    def finish(t, odd, acc):
        base = ((t % H) // 2) * 2 * DH
        cols = _rows(t // H, BQ)
        if odd:
            o = acc * (1.0 / acc[0:1, :])
            even = ot_scr[pl.ds(pl.multiple_of(base + 16, 8), 8), cols]
            o = jnp.concatenate([jnp.where(row8q < 4, even, o[0:8]), o[8:24]], axis=0)
            ot_scr[pl.ds(pl.multiple_of(base + 16, 8), 24), cols] = o
        else:
            ot_scr[pl.ds(pl.multiple_of(base, 8), 24), cols] = acc * (1.0 / acc[23:24, :])

    ms = []
    for g in range(G):
        t = jnp.int32(g)
        q = _unpack(masked_q(t))
        m = None
        for c in range(NC):
            mc = scores(g, tile_of(t), q, c)
            m = mc if m is None else jnp.maximum(m, mc)
        ms.append(jnp.max(m, axis=0, keepdims=True))
        q_cur[g] = masked_q(t + G)
    q_nxt[G - 1] = q_cur[G - 1]
    acc_scr[...] = jnp.ones((24, BQ), F32)
    ot_scr[16:24, 0:BQ] = jnp.zeros((8, BQ), F32)

    for c in late_copies:
        c.wait()
    for g in range(G):
        qt_scr[NX + g, :, 0:BQ] = _pack(w1_ref[g * 128:(g + 1) * 128, 0:BQ])

    def body(j, carry):
        ms, tiles = carry
        new_ms, new_tiles = [], []
        acc = None
        for g in range(G):
            t = j * G + g
            h = t % H
            q = _unpack(q_cur[g])
            prev, acc, mn = acc, None, None
            for c in range(NC):
                p = jnp.exp2(s_scr[g, c * KC:(c + 1) * KC, :] - ms[g]).astype(BF16)
                mc = scores(g, tiles[g], q, c)
                mn = mc if mn is None else jnp.maximum(mn, mc)
                a = _dot(vt_scr[h, :, c * KC:(c + 1) * KC], p)
                acc = a if acc is None else acc + a
                if c == 4:
                    if g == 0:
                        finish(jnp.maximum(t - 1, 1), True, acc_scr[...])
                    else:
                        finish(t - 1, g % 2 == 0, prev)
                if c == 8:
                    q_nxt[g] = masked_q(t + 2 * G)
                if c == 12:
                    q_cur[(g - 1) % G] = q_nxt[(g - 1) % G]
            new_ms.append(jnp.max(mn, axis=0, keepdims=True))
            new_tiles.append(tile_of(t + 2 * G))
        acc_scr[...] = acc
        return tuple(new_ms), tuple(new_tiles)

    jax.lax.fori_loop(0, T // G, body,
                      (tuple(ms), tuple(tile_of(jnp.int32(G + g)) for g in range(G))))
    finish(jnp.int32(T - 1), True, acc_scr[...])

    gw = gw_ref[...].astype(F32).reshape(1, D)

    def ocopy(r):
        return pltpu.make_async_copy(o_buf.at[_rows(r, RB), :], out_hbm.at[_rows(r, RB), :], osem.at[r])

    def final(r, carry):
        xs = x_ref[_rows(r, RB), :]
        h1 = _dot(xs, w1_ref[:, BQ:])
        h0 = _dot(xs[:, G * 128:], w1_ref[G * 128:, 0:BQ])
        for g in range(G):
            h0 = h0 + s_scr[g, _rows(r, RB), :]
        hid = jnp.maximum(jnp.concatenate([h0, h1], axis=1), 0.0).astype(BF16)
        gate = jax.nn.sigmoid(jnp.sum(xs.astype(F32) * gw, axis=-1, keepdims=True))
        o = ot_scr[:, _rows(r, RB)].T.astype(BF16)
        b = _dot(hid, w2_ref[...])
        a = _dot(o, wo_ref[...])
        o_buf[_rows(r, RB), :] = (gate * a + (1.0 - gate) * b).astype(o_buf.dtype)
        ocopy(r).start()
        return carry

    jax.lax.fori_loop(0, NR, final, 0)
    for r in range(NR):
        ocopy(r).wait()


@jax.jit
def pallas_gated_mix__softmax_full_mha__dense_activation_relu__prompt_kernel(
    A_x: jax.Array,
    A_wqkv: jax.Array,
    A_wo: jax.Array,
    B_x: jax.Array,
    B_w1: jax.Array,
    B_w2: jax.Array,
    gate_w: jax.Array,
):
    del B_x
    hbm = pl.BlockSpec(memory_space=pl.ANY)
    out = pl.pallas_call(
        _kernel,
        out_shape=jax.ShapeDtypeStruct((S, D), A_x.dtype),
        in_specs=[hbm] * 6,
        out_specs=hbm,
        scratch_shapes=[
            pltpu.VMEM((D,), BF16),
            pltpu.VMEM((S, D), BF16),
            pltpu.VMEM((D, D), BF16),
            pltpu.VMEM((D, D), BF16),
            pltpu.VMEM((D, D), BF16),
            pltpu.VMEM((D, D), BF16),
            pltpu.VMEM((D, DFF), BF16),
            pltpu.VMEM((DFF, D), BF16),
            pltpu.VMEM((S, D), BF16),
            pltpu.VMEM((D // 2, D), U32),
            pltpu.VMEM((D // 2, D), U32),
            pltpu.VMEM((NX + G, S // 2, 128), U32),
            pltpu.VMEM((NX + G, 64, S), U32),
            pltpu.VMEM((H, 24, S), F32),
            pltpu.VMEM((D, S), F32),
            pltpu.VMEM((G, S, BQ), F32),
            pltpu.VMEM((G, 64, BQ), U32),
            pltpu.VMEM((G, 64, BQ), U32),
            pltpu.VMEM((24, BQ), F32),
            pltpu.SemaphoreType.DMA((len(XCH),)),
            pltpu.SemaphoreType.DMA((7,)),
            pltpu.SemaphoreType.DMA((NR,)),
        ],
        compiler_params=pltpu.CompilerParams(
            vmem_limit_bytes=100 * 1024 * 1024,
            flags={"XLA_TPU_EVENLY_DISTRIBUTE_CRITICAL_NODES": True},
        ),
    )(A_x.reshape(S, D), A_wqkv, A_wo, B_w1, B_w2, gate_w)
    return out.reshape(1, S, D)
```
